```python
import os as _os
_os.environ.setdefault("JAX_PLATFORMS", "cpu")
import jax
import jax.numpy as jnp

def _softmax(x, axis=-1):
    return jax.nn.softmax(x, axis=axis)
def _gelu(x):
    return jax.nn.gelu(x, approximate=True)
def _silu(x):
    return jax.nn.silu(x)
def _sigmoid(x):
    return jax.nn.sigmoid(x)
def _layernorm(x, axis=-1, eps=1e-5):
    m = jnp.mean(x, axis=axis, keepdims=True)
    v = jnp.var(x, axis=axis, keepdims=True)
    return (x - m) / jnp.sqrt(v + eps)
def _scatter_add(tgt, idx, src, axis=0):
    return tgt.at[idx].add(src)
def _segment_sum(src, seg, n):
    return jax.ops.segment_sum(src, seg, n)
class _Rng:
    def __init__(self, key):
        self._k = key
    def _next(self):
        self._k, sub = jax.random.split(self._k)
        return sub
    def normal(self, shape):
        return jax.random.normal(self._next(), shape, dtype=jnp.bfloat16)
    def randint(self, lo, hi, shape):
        return jax.random.randint(self._next(), shape, lo, hi, dtype=jnp.int32)
    def uniform(self, shape, lo=0.0, hi=1.0):
        return jax.random.uniform(self._next(), shape, jnp.bfloat16, lo, hi)
    def permutation(self, n):
        return jax.random.permutation(self._next(), n)


kernel_name = 'gated_mix__ssm_conv_s5__moe_arch_mod__prompt'

def setup_inputs():
    _rng = _Rng(jax.random.key(int.from_bytes(__import__("os").urandom(4), "little")))
    _w = (lambda a: (lambda t: t.astype(jnp.bfloat16) if jnp.issubdtype(t.dtype, jnp.floating) else t)(jnp.asarray(a)))
    def _A_setup():
        B, S, D = 1, 2048, 576
        P = D
        Lambda_re = -0.5 * jnp.exp((lambda *s: _rng.normal(s) * 0.4)(P))
        Lambda_im = (lambda *s: _rng.normal(s) * 0.4)(P) * 1.0
        B_re = (lambda *s: _rng.normal(s) * 0.4)(P, D) * (D ** -0.5)
        B_im = (lambda *s: _rng.normal(s) * 0.4)(P, D) * (D ** -0.5)
        C_re = (lambda *s: _rng.normal(s) * 0.4)(D, P) * (P ** -0.5)
        C_im = (lambda *s: _rng.normal(s) * 0.4)(D, P) * (P ** -0.5)
        log_dt = (lambda *s: _rng.normal(s) * 0.4)(P) * 0.3 - 2.0
        Dskip = (lambda *s: _rng.normal(s) * 0.4)(D)
        return {
            "x": _w((lambda *s: _rng.normal(s) * 0.05)(B, S, D)),
            "Lambda_re": _w(Lambda_re),
            "Lambda_im": _w(Lambda_im),
            "B_re": _w(B_re),
            "B_im": _w(B_im),
            "C_re": _w(C_re),
            "C_im": _w(C_im),
            "log_dt": _w(log_dt),
            "Dskip": _w(Dskip),
        }
    _A_in = _A_setup()

    def _B_setup():
        B, S, D, F, C = 1, 2048, 576, 4608, 2
        return {
            "x": _w((lambda *s: _rng.normal(s) * 0.05)(B, S, D)),
            "w_r": _w((lambda *s: _rng.normal(s) * 1.6)(D)),
            "w_gate": _w((lambda *s: _rng.normal(s) * 0.1)(D, F)),
            "w_up": _w((lambda *s: _rng.normal(s) * 0.1)(D, F)),
            "w_down": _w((lambda *s: _rng.normal(s) * 0.1)(F, D)),
        }
    _B_in = _B_setup()

    return {
        "A_x": _A_in["x"],
        "A_Lambda_re": _A_in["Lambda_re"],
        "A_Lambda_im": _A_in["Lambda_im"],
        "A_B_re": _A_in["B_re"],
        "A_B_im": _A_in["B_im"],
        "A_C_re": _A_in["C_re"],
        "A_C_im": _A_in["C_im"],
        "A_log_dt": _A_in["log_dt"],
        "A_Dskip": _A_in["Dskip"],
        "B_x": _B_in["x"],
        "B_w_r": _B_in["w_r"],
        "B_w_gate": _B_in["w_gate"],
        "B_w_up": _B_in["w_up"],
        "B_w_down": _B_in["w_down"],
        "gate_w": _w((lambda *s: _rng.normal(s) * 0.05)(576) * 16.0),
    }

def reference(A_x, A_Lambda_re, A_Lambda_im, A_B_re, A_B_im, A_C_re, A_C_im, A_log_dt, A_Dskip, B_x, B_w_r, B_w_gate, B_w_up, B_w_down, gate_w):
    def _A_ref(x, Lambda_re, Lambda_im, B_re, B_im, C_re, C_im, log_dt, Dskip):
        Bsz, L, H = x.shape
        Lam = Lambda_re + 1j * Lambda_im
        Bmat = B_re + 1j * B_im
        Cmat = C_re + 1j * C_im
        dt = jnp.exp(log_dt)
        Lam_bar = jnp.exp(dt * Lam)
        B_bar = ((Lam_bar - 1.0) / Lam)[:, None] * Bmat
        Bu = jnp.einsum("bld,pd->blp", x + 0j, B_bar)
        h = jnp.zeros_like(Bu[:, 0, :])
        hs = []
        for t in range(L):
            h = Lam_bar[None, :] * h + Bu[:, t, :]
            hs.append(h)
        hseq = jnp.stack(hs, 1)
        y = 2.0 * jnp.einsum("blp,dp->bld", hseq, Cmat).real + x * Dskip[None, None, :]
        return y

    def _B_ref(x, w_r, w_gate, w_up, w_down):
        B, S, D = x.shape
        C = 2
        r = x @ w_r
        idx = jnp.argsort(-r, axis=-1)[:, :C]
        idx_e = jnp.repeat(idx.reshape(B, C, 1), D, axis=2)
        x_sel = jnp.take_along_axis(x, idx_e, axis=1)
        g = _silu(x_sel @ w_gate)
        u = x_sel @ w_up
        y = (g * u) @ w_down
        r_sel = _sigmoid(jnp.take_along_axis(r, idx, axis=1))
        y = y * r_sel.reshape(B, C, 1)
        b_off = (jnp.arange(B) * S).reshape(B, 1)
        flat_idx = (idx + b_off).reshape(B * C)
        zero = (x * 0.0).reshape(B * S, D)
        upd = _scatter_add(zero, flat_idx, y.reshape(B * C, D), axis=0)
        return x + upd.reshape(B, S, D)

    x = A_x
    g = _sigmoid((x * gate_w).sum(-1, keepdims=True))
    a = _A_ref(x, A_Lambda_re, A_Lambda_im, A_B_re, A_B_im, A_C_re, A_C_im, A_log_dt, A_Dskip)
    b = _B_ref(x, B_w_r, B_w_gate, B_w_up, B_w_down)
    return g * a + (1 - g) * b
```

```python
import functools

import jax
import jax.numpy as jnp
from jax import lax
import jax.experimental.pallas as pl
import jax.experimental.pallas.tpu as pltpu

f32 = jnp.float32
bf16 = jnp.bfloat16
u32 = jnp.uint32

_NN = (((1,), (0,)), ((), ()))
_NT = (((1,), (1,)), ((), ()))
_TN = (((0,), (0,)), ((), ()))
LANES = 128


def _dot(a, b, dims):
    return lax.dot_general(a, b, dims, preferred_element_type=f32)


def _cmul(ar, ai, br, bi):
    return ar * br - ai * bi, ar * bi + ai * br


def _round_bf16(v):
    return v.astype(bf16).astype(f32)


def _sigmoid(v):
    return 1.0 / (1.0 + jnp.exp(-v))


def _kernel(x_h, lre_h, lim_h, bre_h, bim_h, cre_h, cim_h, ldt_h, dsk_h, wr_h, wg_h, wu_h, wd_h, gw_h,
            o_h,
            x_v, lre_v, lim_v, ldt_v, dsk_v, wr_v, gw_v, b_v, cre_v, cim_v, cp_v, wg_v, wu_v, wd_v,
            xw_v, xp_v, bu_v, hw_v, o_v, gr_v, dcol_v, sem_in, sem_out, *, T, SYNC):
    D, L = x_v.shape
    NC = L // T
    TS = T // 8
    HS = TS // 2
    DF = (D // LANES) * LANES
    DR = D - DF
    NT_ = L // LANES
    TPC = T // LANES

    n_sem = [0]

    def copy(src, dst):
        c = pltpu.make_async_copy(src, dst, sem_in.at[n_sem[0]])
        n_sem[0] += 1
        return c

    cx = [copy(x_h.at[:, pl.ds(c * T, T)], x_v.at[:, pl.ds(c * T, T)]) for c in range(NC)]
    cb = [copy(bre_h.at[pl.ds(0, DF)], b_v.at[pl.ds(0, DF)]),
          copy(bim_h.at[pl.ds(0, DF)], b_v.at[pl.ds(DF, DF)]),
          copy(bre_h.at[pl.ds(DF, DR)], b_v.at[pl.ds(2 * DF, DR)]),
          copy(bim_h.at[pl.ds(DF, DR)], b_v.at[pl.ds(2 * DF + DR, DR)])]
    cv = [copy(s, d) for s, d in ((lre_h, lre_v), (lim_h, lim_v), (ldt_h, ldt_v), (dsk_h, dsk_v),
                                  (wr_h, wr_v), (gw_h, gw_v))]
    cc = [copy(cre_h, cre_v), copy(cim_h, cim_v)]
    cw = [copy(wg_h, wg_v), copy(wu_h, wu_v), copy(wd_h, wd_v)]

    cx[0].start()
    for c in cv:
        c.start()
    for c in cb:
        c.start()

    def row(ref):
        return ref[...].astype(f32).reshape(1, D)

    for c in cv:
        c.wait()
    cx[1].start()
    for c in cc:
        c.start()

    l_re, l_im = row(lre_v), row(lim_v)
    dt = _round_bf16(jnp.exp(row(ldt_v)))
    mag = jnp.exp(dt * l_re)
    lam_r = mag * jnp.cos(dt * l_im)
    lam_i = mag * jnp.sin(dt * l_im)
    sc = jnp.maximum(jnp.abs(l_re), jnp.abs(l_im))
    a, b = l_re / sc, l_im / sc
    den = (a * a + b * b) * sc
    f_r = 2.0 * ((lam_r - 1.0) * a + lam_i * b) / den
    f_i = 2.0 * (lam_i * a - (lam_r - 1.0) * b) / den
    ar = jnp.broadcast_to(jnp.concatenate([lam_r, lam_r[:, DF:]], axis=1), (8, DF + LANES))
    ai = jnp.broadcast_to(jnp.concatenate([lam_i, -lam_i[:, DF:]], axis=1), (8, DF + LANES))
    pr, pi = ar, ai
    for _ in range(TS.bit_length() - 1):
        pr, pi = _cmul(pr, pi, pr, pi)
    seg_pows = [(pr, pi)]
    for _ in range(2):
        pr, pi = _cmul(pr, pi, pr, pi)
        seg_pows.append((pr, pi))
    sub = lax.broadcasted_iota(jnp.int32, (8, DF + LANES), 0)

    dsk = jnp.concatenate([row(dsk_v), jnp.zeros((1, LANES - DR), f32)], axis=1)
    dcol_v[...] = jnp.transpose(jnp.broadcast_to(dsk, (LANES, DF + LANES)))[:D]
    rid = lax.broadcasted_iota(jnp.int32, (16, D), 0)
    w2 = jnp.where(rid == 0, row(gw_v), jnp.where(rid == 8, row(wr_v), 0.0)).astype(bf16)

    def stage_x(c):
        s = c % 2
        for k in range(DF // LANES + 1):
            if k < DF // LANES:
                blk = x_v[pl.ds(k * LANES, LANES), pl.ds(c * T, T)]
            else:
                blk = jnp.concatenate([x_v[pl.ds(DF, DR), pl.ds(c * T, T)], jnp.zeros((LANES - DR, T), bf16)], axis=0)
            xw_v[s, k] = pltpu.bitcast(jnp.transpose(blk), u32)
        for i in range(HS):
            w = jnp.concatenate([xw_v[s, k, pl.ds(i, 8, stride=HS), :] for k in range(DF // LANES + 1)], axis=1)
            lo = lax.bitcast_convert_type(w << 16, f32)
            hi = lax.bitcast_convert_type(w & jnp.uint32(0xFFFF0000), f32)
            xp_v[s, pl.ds(16 * i, 16), :] = jnp.concatenate([lo, hi], axis=0).astype(bf16)
        gr_v[:, pl.ds(c * T, T)] = _dot(w2, x_v[:, pl.ds(c * T, T)], _NN)

    def stage_m1(c):
        s = c % 2
        bu_v[s] = _dot(xp_v[s, :, pl.ds(0, D)], b_v[...], _NT)

    def load_u(s, j):
        u = bu_v[s, pl.ds(8 * j, 8), :]
        t = u[:, 2 * DF:]
        return (jnp.concatenate([u[:, :DF], t], axis=1),
                jnp.concatenate([u[:, DF:2 * DF], pltpu.roll(t, DR, 1)], axis=1))

    def step(s, j, hr, hi):
        ur, ui = load_u(s, j)
        return ar * hr - ai * hi + ur, ar * hi + ai * hr + ui

    def stage_scan(c, carry):
        s = c % 2
        er, ei = load_u(s, 0)
        for j in range(1, TS):
            er, ei = step(s, j, er, ei)
        vr = jnp.where(sub == 0, carry[0], pltpu.roll(er, 1, 0))
        vi = jnp.where(sub == 0, carry[1], pltpu.roll(ei, 1, 0))
        for n, (qr, qi) in enumerate(seg_pows):
            sh = 1 << n
            tr = jnp.where(sub >= sh, pltpu.roll(vr, sh, 0), 0.0)
            ti = jnp.where(sub >= sh, pltpu.roll(vi, sh, 0), 0.0)
            mr, mi = _cmul(qr, qi, tr, ti)
            vr, vi = vr + mr, vi + mi
        mr, mi = _cmul(seg_pows[0][0], seg_pows[0][1], vr, vi)
        new_carry = (pltpu.roll(mr + er, 1, 0), pltpu.roll(mi + ei, 1, 0))
        hr, hi = vr, vi
        for i in range(HS):
            h0r, h0i = step(s, 2 * i, hr, hi)
            hr, hi = step(s, 2 * i + 1, h0r, h0i)
            h0 = jnp.concatenate([h0r[:, :DF], h0i[:, :DF], h0r[:, DF:]], axis=1)
            h1 = jnp.concatenate([hr[:, :DF], hi[:, :DF], hr[:, DF:]], axis=1)
            q = lax.bitcast_convert_type(_round_bf16(jnp.concatenate([h0, h1], axis=0)), u32)
            w = (q[:8] >> 16) | q[8:]
            for k in range(hw_v.shape[1]):
                hw_v[s, k, pl.ds(i, 8, stride=HS), :] = w[:, k * LANES:(k + 1) * LANES]
        return new_carry

    def stage_c():
        cr, ci = cre_v[...].astype(f32), cim_v[...].astype(f32)
        g_r = cr * f_r - ci * f_i
        g_i = -(cr * f_i + ci * f_r)
        cp_v[...] = jnp.concatenate([g_r[:, :DF], g_i[:, :DF], g_r[:, DF:], g_i[:, DF:]], axis=1).astype(bf16)

    def stage_m2(c):
        s = c % 2
        h = jnp.concatenate([pltpu.bitcast(hw_v[s, k], bf16) for k in range(hw_v.shape[1])], axis=1)
        y = _dot(cp_v[...], h, _NT)
        g = _round_bf16(_sigmoid(_round_bf16(gr_v[pl.ds(0, 1), pl.ds(c * T, T)])))
        for t in range(TPC):
            sl = slice(t * LANES, (t + 1) * LANES)
            gt = g[:, sl]
            xt = x_v[:, pl.ds(c * T + t * LANES, LANES)].astype(f32)
            o_v[c * TPC + t] = gt * y[:, sl] + xt * (gt * dcol_v[...] + (1.0 - gt))

    def out_copy(t):
        off = t * LANES if isinstance(t, int) else pl.multiple_of(t * LANES, LANES)
        return pltpu.make_async_copy(o_v.at[t], o_h.at[:, pl.ds(off, LANES)], sem_out.at[0])

    def select():
        r = _round_bf16(gr_v[pl.ds(8, 1), :])
        r = jnp.where(r == r, r, -jnp.inf)
        pos = lax.broadcasted_iota(jnp.int32, r.shape, 1).astype(f32)
        m0 = jnp.max(r, axis=1, keepdims=True)
        i0 = jnp.min(jnp.where(r == m0, pos, float(L)), axis=1, keepdims=True)
        r1 = jnp.where(pos == i0, -jnp.inf, r)
        m1 = jnp.max(r1, axis=1, keepdims=True)
        i1 = jnp.min(jnp.where((r1 == m1) & (pos != i0), pos, float(L)), axis=1, keepdims=True)
        return (m0, m1), (i0, i1), (i0.astype(jnp.int32)[0, 0], i1.astype(jnp.int32)[0, 0])

    cx[0].wait()
    stage_x(0)
    for c in cb:
        c.wait()
    for c in cx[2:]:
        c.start()
    for c in cw:
        c.start()
    stage_m1(0)
    carry = (jnp.zeros((8, DF + LANES), f32), jnp.zeros((8, DF + LANES), f32))
    tiles = None
    for c in range(NC):
        if c + 1 < NC:
            cx[c + 1].wait()
            stage_x(c + 1)
            stage_m1(c + 1)
        if c == 0:
            for d in cc:
                d.wait()
            stage_c()
        if c == NC - 2:
            vals, idxf, idx = select()
            tiles = [jnp.clip(i // LANES, 0, NT_ - 1) for i in idx]
        carry = stage_scan(c, carry)
        if c == SYNC:
            for d in cw:
                d.wait()
            for t in range(c * TPC):
                @pl.when((tiles[0] != t) & (tiles[1] != t))
                def _():
                    out_copy(t).start()
        stage_m2(c)
        if c >= SYNC:
            for t in range(c * TPC, (c + 1) * TPC):
                @pl.when((tiles[0] != t) & (tiles[1] != t))
                def _():
                    out_copy(t).start()

    lane = lax.broadcasted_iota(jnp.int32, (16, LANES), 1)
    rw = lax.broadcasted_iota(jnp.int32, (16, LANES), 0)
    xs = jnp.zeros((16, D), f32)
    hots = []
    for n in range(2):
        off = pl.multiple_of(tiles[n] * LANES, LANES)
        hot = ((lane == idx[n] - off) & (rw == n)).astype(f32)
        hots.append(hot)
        xs = xs + _dot(hot.astype(bf16), x_v[:, pl.ds(off, LANES)], _NT)
    xs = xs.astype(bf16)
    gt = _round_bf16(_dot(xs, wg_v[...], _NN))
    up = _round_bf16(_dot(xs, wu_v[...], _NN))
    hid = (_round_bf16(gt * _sigmoid(gt)) * up).astype(bf16)
    y = _dot(hid, wd_v[...], _NT).astype(bf16)
    for n in range(2):
        off = pl.multiple_of(tiles[n] * LANES, LANES)
        g = _round_bf16(_sigmoid(_round_bf16(gr_v[pl.ds(0, 1), pl.ds(off, LANES)])))
        scale = (1.0 - g) * _round_bf16(_sigmoid(vals[n]))
        o_v[tiles[n]] = o_v[tiles[n]] + scale * _dot(y, hots[n].astype(bf16), _TN)
    out_copy(tiles[0]).start()

    @pl.when(tiles[1] != tiles[0])
    def _():
        out_copy(tiles[1]).start()

    pltpu.make_async_copy(o_v, o_v, sem_out.at[0]).wait()


def build(T=256, SYNC=None, interpret=False, name="gm", **cp):
    def fn(A_x, A_Lambda_re, A_Lambda_im, A_B_re, A_B_im, A_C_re, A_C_im, A_log_dt, A_Dskip,
           B_x, B_w_r, B_w_gate, B_w_up, B_w_down, gate_w):
        _, L, D = A_x.shape
        F = B_w_gate.shape[1]
        NC = L // T
        KT = pl.cdiv(D, LANES)
        vm = pltpu.VMEM
        out = pl.pallas_call(
            functools.partial(_kernel, T=T, SYNC=NC - 1 if SYNC is None else SYNC),
            in_specs=[pl.BlockSpec(memory_space=pl.ANY)] * 14,
            out_specs=pl.BlockSpec(memory_space=pl.ANY),
            out_shape=jax.ShapeDtypeStruct((D, L), f32),
            scratch_shapes=[
                vm((D, L), bf16)] + [vm((D,), bf16)] * 6 + [
                vm((2 * D, D), bf16), vm((D, D), bf16), vm((D, D), bf16), vm((D, 2 * D), bf16),
                vm((D, F), bf16), vm((D, F), bf16), vm((D, F), bf16),
                vm((2, KT, T // 2, LANES), u32), vm((2, T, KT * LANES), bf16), vm((2, T, 2 * D), f32),
                vm((2, 2 * D // LANES, T // 2, LANES), u32),
                vm((L // LANES, D, LANES), f32), vm((16, L), f32), vm((D, LANES), f32),
                pltpu.SemaphoreType.DMA((NC + 15,)), pltpu.SemaphoreType.DMA((1,)),
            ],
            compiler_params=pltpu.CompilerParams(
                vmem_limit_bytes=100 * 1024 * 1024, disable_semaphore_checks=True, disable_bounds_checks=True, **cp),
            interpret=interpret,
            name=name,
        )(jnp.transpose(A_x[0]), A_Lambda_re, A_Lambda_im, A_B_re, A_B_im, A_C_re, A_C_im, A_log_dt, A_Dskip,
          B_w_r, B_w_gate, B_w_up, jnp.transpose(B_w_down), gate_w)
        return jnp.transpose(out)[None]
    return fn


@jax.jit
def pallas_gated_mix__ssm_conv_s5__moe_arch_mod__prompt_kernel(
        A_x, A_Lambda_re, A_Lambda_im, A_B_re, A_B_im, A_C_re, A_C_im, A_log_dt, A_Dskip,
        B_x, B_w_r, B_w_gate, B_w_up, B_w_down, gate_w):
    return build(T=256)(A_x, A_Lambda_re, A_Lambda_im, A_B_re, A_B_im, A_C_re, A_C_im, A_log_dt, A_Dskip,
                     B_x, B_w_r, B_w_gate, B_w_up, B_w_down, gate_w)
```

```python
import functools

import jax
import jax.numpy as jnp
from jax import lax
import jax.experimental.pallas as pl
import jax.experimental.pallas.tpu as pltpu

f32 = jnp.float32
bf16 = jnp.bfloat16
u32 = jnp.uint32

LANES = 128
SUBS = 8
NMXU = 4
WIDE = NMXU * LANES

T = 256
PAIRS = T // SUBS // 2
PITCH = PAIRS + 1
ROWS = 144
WARM = 3
LATE = 2
WAYS = 2
TAIL = 48

X_AT = 38
W_AT = (84, 137, 180, 196)

_NN = (((1,), (0,)), ((), ()))
_NT = (((1,), (1,)), ((), ()))


def _dot(a, b, dims, acc=None):
    d = lax.dot_general(a, b, dims, preferred_element_type=f32)
    return d if acc is None else d + acc


def _cmul(ar, ai, br, bi):
    return ar * br - ai * bi, ar * bi + ai * br


def _round_bf16(v):
    return v.astype(bf16).astype(f32)


def _sigmoid(v):
    return 1.0 / (1.0 + jnp.exp(-v))


def _pack(lo, hi):
    lo, hi = (lax.bitcast_convert_type(_round_bf16(v), u32) for v in (lo, hi))
    return (lo >> 16) | hi


def _unpack(w):
    return (lax.bitcast_convert_type(w << 16, f32),
            lax.bitcast_convert_type(w & jnp.uint32(0xFFFF0000), f32))


def _column(v):
    return jnp.transpose(jnp.broadcast_to(v, (LANES, LANES)))


def _kernel(x_h, lre_h, lim_h, bre_h, bim_h, cre_h, cim_h, ldt_h, dsk_h, wr_h, wg_h, wu_h, wd_h, gw_h, o_h,
            x_v, vec_v, b_v, cre_v, cim_v, c_v, wg_v, wu_v, wd_v, xw_v, u_v, hw_v, o_v, fix_v, g_v,
            sem_in, sem_out):
    D, L = x_v.shape
    F = wg_v.shape[1]
    NF = D // LANES
    DF = NF * LANES
    DR = D - DF
    NP = NF + 1
    NK = 2 * NF + 1
    NTILE = L // LANES
    size = [LANES] * NF + [DR]
    first = [k * LANES for k in range(NF)] + [D - LANES]

    copies = []

    def fetch(src, dst, idx=None):
        if idx is not None:
            src, dst = src.at[idx], dst.at[idx]
        copies.append(pltpu.make_async_copy(src, dst, sem_in.at[len(copies)]))
        copies[-1].start()
        return copies[-1]

    def span(lo, hi):
        return pl.ds(lo, hi - lo)

    def wait(*group):
        for c in group:
            c.wait()

    got_vec = [fetch(s, d) for s, d in zip((lre_h, lim_h, ldt_h, dsk_h, wr_h, gw_h), vec_v)]
    got_x = [fetch(x_h, x_v, (slice(None), span(0, 2 * T)))]
    got_b = [[fetch(src.at[pl.ds(p * LANES, size[p])], b_v.at[pl.ds(2 * p * LANES + i * size[p], size[p])])
              for i, src in enumerate((bre_h, bim_h))] for p in range(NP)]
    got_x += [fetch(x_h, x_v, (slice(None), s)) for s in (span(2 * T, 4 * T), span(4 * T, L))]
    got_w = [[fetch(cre_h, cre_v), fetch(cim_h, cim_v), fetch(wg_h, wg_v), fetch(wu_h, wu_v, span(DF - LANES, D))],
             [fetch(wu_h, wu_v, span(0, DF - LANES)), fetch(wd_h, wd_v, span(0, LANES))],
             [fetch(wd_h, wd_v, span(LANES, D - TAIL))],
             [fetch(wd_h, wd_v, span(D - TAIL, D))]]

    wait(*got_vec)
    l_re, l_im, log_dt, skip, w_r, gate_w = (v[...].astype(f32).reshape(1, D) for v in vec_v)
    dt = _round_bf16(jnp.exp(log_dt))
    mag = jnp.exp(dt * l_re)
    lam_r = mag * jnp.cos(dt * l_im)
    lam_i = mag * jnp.sin(dt * l_im)
    big = jnp.maximum(jnp.abs(l_re), jnp.abs(l_im))
    a, b = l_re / big, l_im / big
    den = (a * a + b * b) * big
    f_r = 2.0 * ((lam_r - 1.0) * a + lam_i * b) / den
    neg_f_i = -2.0 * (lam_i * a - (lam_r - 1.0) * b) / den

    def mode_tiles(v, v_last):
        v = jnp.concatenate([v, v_last], axis=1)
        return jnp.stack([jnp.broadcast_to(v[:, p * LANES:(p + 1) * LANES], (SUBS, LANES)) for p in range(NP)])

    lam = mode_tiles(lam_r, lam_r[:, DF:]), mode_tiles(lam_i, -lam_i[:, DF:])
    powers = [lam]
    for _ in range((T // 2).bit_length() - 1):
        powers.append(_cmul(*powers[-1], *powers[-1]))
    powers = powers[-3:]

    sub = lax.broadcasted_iota(jnp.int32, (SUBS, LANES), 0)
    lane = lax.broadcasted_iota(jnp.int32, (SUBS, LANES), 1)
    score_w = [jnp.where(sub == 0, gate_w[:, k:k + LANES], jnp.where(sub == 1, w_r[:, k:k + LANES], 0.0))
               for k in first]
    score_w[NF] = jnp.where(lane >= LANES - DR, score_w[NF], 0.0)
    skip = jnp.concatenate([_column(skip[:, k:k + LANES])[LANES - n:] for k, n in zip(first, size)], axis=0)

    def reorder_x(c):
        words = []
        for k in range(NP):
            blk = x_v[pl.ds(k * LANES, size[k]), pl.ds(c * T, T)]
            if k == NF:
                blk = jnp.concatenate([blk, jnp.zeros((LANES - DR, T), bf16)], axis=0)
            words.append(pltpu.bitcast(jnp.transpose(blk), u32))
        words = jnp.stack(words)
        for s in range(SUBS):
            xw_v[c][:, pl.ds(s * PITCH, PAIRS), :] = words[:, s * PAIRS:(s + 1) * PAIRS]
        rows = []
        for i in range(PAIRS):
            rows += _unpack(xw_v[c][:, pl.ds(i, SUBS, stride=PITCH), :])
        rows = jnp.concatenate(rows, axis=1).astype(bf16)
        return [rows[k, :, :size[k]] for k in range(NP)]

    carry = [(0.0, 0.0)] * NP

    def scan(c, p, u):
        u_v[c % 2, p, 0] = u[2 * p]
        u_v[c % 2, p, 1] = u[2 * p + 1] if p < NF else pltpu.roll(u[2 * p], DR, 1)
        lr, li = lam[0][p], lam[1][p]

        def two_steps(i, h):
            v = u_v[c % 2, p, :, pl.ds(2 * SUBS * i, 2 * SUBS), :]
            h0 = lr * h[0] - li * h[1] + v[0, :SUBS], lr * h[1] + li * h[0] + v[1, :SUBS]
            return h0, (lr * h0[0] - li * h0[1] + v[0, SUBS:], lr * h0[1] + li * h0[0] + v[1, SUBS:])

        def emit(i, h):
            h0, h1 = two_steps(i, h)
            for j in range(2 if p < NF else 1):
                hw_v[c][2 * p + j, pl.ds(i, SUBS, stride=PITCH), :] = _pack(h0[j], h1[j])
            return h1

        zero = jnp.zeros((SUBS, LANES), f32)
        h = lax.fori_loop(0, PAIRS, lambda i, h: two_steps(i, h)[1], (zero, zero), unroll=True)
        h = [jnp.where(sub == 0, prev, pltpu.roll(v, 1, 0)) for v, prev in zip(h, carry[p])]
        for n, (qr, qi) in enumerate(powers):
            m = _cmul(qr[p], qi[p], *[jnp.where(sub >= 1 << n, pltpu.roll(v, 1 << n, 0), 0.0) for v in h])
            h = h[0] + m[0], h[1] + m[1]
        carry[p] = [pltpu.roll(v, 1, 0) for v in lax.fori_loop(0, PAIRS, emit, h, unroll=True)]

    def scale_c(m0):
        for p in range(NP):
            sl = slice(p * LANES, p * LANES + size[p])
            cr = cre_v[pl.ds(m0, ROWS), sl].astype(f32)
            ci = cim_v[pl.ds(m0, ROWS), sl].astype(f32)
            parts = [cr * f_r[:, sl] + ci * neg_f_i[:, sl], cr * neg_f_i[:, sl] - ci * f_r[:, sl]]
            if p == NF:
                parts = [jnp.concatenate(parts, axis=1)]
            for k, v in enumerate(parts, 2 * p):
                c_v[k, pl.ds(m0 // 2, ROWS // 2), :] = pltpu.bitcast(v.astype(bf16), u32)

    def mix(t, m0, y):
        g = g_v[pl.ds(0, 1), pl.ds(t * LANES, LANES)]
        x = x_v[pl.ds(m0, ROWS), pl.ds(t * LANES, LANES)].astype(f32)
        out = g * y + x * (g * skip[m0:m0 + ROWS] + (1.0 - g))
        if t >= NTILE - LATE:
            if "y" not in routed:
                finish_routed()
            out = out + routed_update(t * LANES, m0, ROWS)
        o_v[t, pl.ds(m0 // (WAYS * SUBS), ROWS // (WAYS * SUBS))] = out.reshape(-1, WAYS, SUBS, LANES)
        if m0 + ROWS == D:
            finished.append(t)
            if n_group[0] >= W_AT[2]:
                release()

    finished = []

    def write(src, off):
        for e in range(WAYS):
            pltpu.make_async_copy(src.at[:, e], o_h.at[:, e, :, pl.ds(off, LANES)], sem_out.at[0]).start()

    def release():
        for t in finished:
            if t >= NTILE - LATE:
                write(o_v.at[t], t * LANES)
            else:
                pl.when((routed["tile"][0] != t) & (routed["tile"][1] != t))(
                    functools.partial(write, o_v.at[t], t * LANES))
        finished.clear()

    def routed_update(off, m0, rows):
        gs = g_v[:, pl.ds(off, LANES)]
        y0, y1 = _unpack(routed["y"][m0:m0 + rows])
        pos = lane[0:1] + off
        y = jnp.where(pos == routed["idx"][0], y0, jnp.where(pos == routed["idx"][1], y1, 0.0))
        return (1.0 - gs[0:1]) * gs[1:2] * y

    def finish_routed():
        while thin:
            thin_step()
        routed["y"] = jnp.concatenate(
            [_column(_pack(y[0:1], y[1:2]))[LANES - n:] for y, n in zip(down, size)], axis=0)
        for n, tile in enumerate(routed["tile"]):
            t = jnp.minimum(tile, NTILE - LATE - 1)
            off = pl.multiple_of(t * LANES, LANES)
            fix_v[n] = o_v[t] + routed_update(off, 0, D).reshape(fix_v.shape[1:])
            held = tile < NTILE - LATE
            pl.when(held if n == 0 else held & (tile != routed["tile"][0]))(
                functools.partial(write, fix_v.at[n], off))

    routed = {}
    scores = []
    gate, up, hidden, down = {}, {}, {}, []

    def score(lo, hi):
        for t0 in range(lo, hi, WIDE):
            acc = None
            for k in range(NP):
                acc = _dot(score_w[k], x_v[pl.ds(first[k], LANES), pl.ds(t0, WIDE)], _NN, acc)
                if k == NF:
                    acc = _round_bf16(acc)
                    g_v[:, pl.ds(t0, WIDE)] = _round_bf16(_sigmoid(acc))
                    scores.append(acc[1:2])
                yield

    def route():
        r = jnp.concatenate(scores, axis=1)
        r = jnp.where(r == r, r, -jnp.inf)
        pos = lax.broadcasted_iota(jnp.int32, r.shape, 1).astype(f32)
        i0 = jnp.min(jnp.where(r == jnp.max(r, axis=1, keepdims=True), pos, float(L)), axis=1, keepdims=True)
        r = jnp.where(pos == i0, -jnp.inf, r)
        i1 = jnp.min(jnp.where((r == jnp.max(r, axis=1, keepdims=True)) & (pos != i0), pos, float(L)),
                     axis=1, keepdims=True)
        routed["idx"] = [jnp.clip(i.astype(jnp.int32)[0, 0], 0, L - 1) for i in (i0, i1)]
        routed["tile"] = [lax.shift_right_logical(i, LANES.bit_length() - 1) for i in routed["idx"]]
        for _ in range(6):
            yield
        off = [pl.multiple_of(t * LANES, LANES) for t in routed["tile"]]
        hot = [((lane + off[n] == routed["idx"][n]) & (sub == n)).astype(f32) for n in range(2)]
        head = None
        for n in range(2):
            head = _dot(hot[n], x_v[pl.ds(0, DF), pl.ds(off[n], LANES)], _NT, head)
            yield
        rest = None
        for n in range(2):
            xr = x_v[pl.ds(DF, DR), pl.ds(off[n], LANES)]
            z = jnp.zeros_like(xr)
            rest = _dot(hot[n], jnp.concatenate([xr, z], axis=0), _NT, rest)
            rest = _dot(pltpu.roll(hot[n], 2, 0), jnp.concatenate([z, xr], axis=0), _NT, rest)
        routed["x"] = [head[:, k * LANES:(k + 1) * LANES] for k in range(NF)] + [rest]
        yield

    def project_rest():
        for j in range(0, F, WIDE):
            w = jnp.concatenate([w_v[pl.ds(DF, DR), pl.ds(j, WIDE)] for w_v in (wg_v, wu_v)], axis=0)
            gate[j] = _dot(routed["x"][NF], w, _NN)
            up[j] = pltpu.roll(gate[j], SUBS - 2, 0)
            yield

    def project(w_v, acc, ks):
        for j in range(0, F, WIDE):
            for k in ks:
                acc[j] = _dot(routed["x"][k], w_v[pl.ds(k * LANES, LANES), pl.ds(j, WIDE)], _NN, acc[j])
                yield

    def project_down(ks):
        for k in ks:
            acc = None
            for j in range(0, F, WIDE):
                if j not in hidden:
                    g = _round_bf16(gate[j])
                    hidden[j] = _round_bf16(_round_bf16(g * _sigmoid(g)) * _round_bf16(up[j]))
                acc = _dot(hidden[j], wd_v[pl.ds(first[k], LANES), pl.ds(j, WIDE)], _NT, acc)
                yield
            down.append(acc)

    ffn = [[project_rest(), project(wg_v, gate, range(NF)), project(wu_v, up, [NF - 1])],
           [project(wu_v, up, range(NF - 1)), project_down([0])],
           [project_down(range(1, NF))],
           [project_down([NF])]]
    thin = []

    def thin_step():
        while thin:
            if next(thin[0], 0) is None:
                return
            thin.pop(0)

    x_rows = {}
    inputs = {}

    def state_inputs(passes):
        left = len(passes) % NMXU
        for i, (c, n, k) in enumerate(passes):
            if c not in x_rows:
                x_rows[c] = reorder_x(c)
            w = b_v[pl.ds(n * LANES, LANES), pl.ds(k * LANES, size[k])]
            u = inputs.setdefault(c, {})
            if i >= len(passes) - left:
                r = T * left // NMXU
                u[n] = jnp.concatenate([_dot(x_rows[c][k][q:q + r], w, _NT) for q in range(0, T, r)], axis=0) + u[n]
            else:
                u[n] = _dot(x_rows[c][k], w, _NT, u.get(n))
            if k == NF and (n % 2 or n == NK - 1):
                done.append(functools.partial(scan, c, n // 2, u))
            if i % NMXU == NMXU - 1:
                yield True
        if left:
            yield False

    def state_outputs(pieces):
        per_tile = SUBS * LANES // T
        h = {}
        for i, (t, m0) in enumerate(pieces):
            if t not in h:
                c, tt = divmod(t, T // LANES)
                w = jnp.concatenate([hw_v[c][:, pl.ds((tt * per_tile + s) * PITCH, PAIRS), :]
                                     for s in range(per_tile)], axis=1)
                w = pltpu.bitcast(w, bf16)
                h[t] = [w[k] for k in range(NK)]
            if t == 0:
                scale_c(m0)
            lhs = pltpu.bitcast(c_v[:, pl.ds(m0 // 2, ROWS // 2), :], bf16)
            acc = None
            for k in range(NK):
                acc = _dot(lhs[k], h[t][k], _NT, acc)
                if k == NK - 1:
                    done.append(functools.partial(mix, t, m0, acc))
                if (i * NK + k) % NMXU == NMXU - 1:
                    yield True

    done, later = [], []
    n_group = [0]

    def consume():
        for fn in later:
            fn()
        later[:] = done
        done.clear()

    def run(groups):
        for full in groups:
            if full:
                thin_step()
            consume()
            n_group[0] += 1
            if n_group[0] == X_AT:
                wait(got_x[2])
                thin.extend([score(4 * T, L), route()])
            if n_group[0] in W_AT:
                n = W_AT.index(n_group[0])
                wait(*got_w[n])
                thin.extend(ffn[n])
                if n == 2:
                    release()

    wait(got_x[0])
    x_rows[0] = reorder_x(0)
    wait(*got_b[0])
    run(state_inputs([(c, n, k) for c in (0, 1) for n in (0, 1) for k in range(NP)]))
    wait(*got_b[1], *got_b[2])
    run(state_inputs([(c, n, k) for ns in ((2, 3), (4, 5)) for c in (0, 1) for n in ns for k in range(NP)]))
    wait(*got_b[3], *got_b[4], got_x[1])
    thin.append(score(0, 4 * T))
    run(state_inputs([(c, n, k) for ns in ((6, 7), (8,)) for c in (0, 1) for n in ns for k in range(NP)]))
    order = [(n, k) for k in range(NP) for n in range(2)] + [(n, k) for n in range(2, NK) for k in range(NP)]
    run(state_inputs([(c, n, k) for c in range(2, L // T) for n, k in order]))
    run(state_outputs([(t, m0) for m0 in range(0, D, ROWS) for t in range(WARM)]
                      + [(t, m0) for t in range(WARM, NTILE) for m0 in range(0, D, ROWS)]))
    consume()
    pltpu.make_async_copy(o_h, o_h, sem_out.at[0]).wait()


@jax.jit
def pallas_gated_mix__ssm_conv_s5__moe_arch_mod__prompt_kernel(
    A_x: jax.Array,
    A_Lambda_re: jax.Array,
    A_Lambda_im: jax.Array,
    A_B_re: jax.Array,
    A_B_im: jax.Array,
    A_C_re: jax.Array,
    A_C_im: jax.Array,
    A_log_dt: jax.Array,
    A_Dskip: jax.Array,
    B_x: jax.Array,
    B_w_r: jax.Array,
    B_w_gate: jax.Array,
    B_w_up: jax.Array,
    B_w_down: jax.Array,
    gate_w: jax.Array,
):
    del B_x
    assert A_x.shape == (1, 2048, 576) and B_w_gate.shape == (576, 4608), "the schedule is laid out for these sizes"
    _, L, D = A_x.shape
    F = B_w_gate.shape[1]
    vmem = pltpu.VMEM
    feature_tiles, state_tiles = pl.cdiv(D, LANES), 2 * D // LANES
    out_rows = (D // (WAYS * SUBS), WAYS, SUBS)
    out = pl.pallas_call(
        _kernel,
        in_specs=[pl.BlockSpec(memory_space=pl.ANY)] * 14,
        out_specs=pl.BlockSpec(memory_space=pl.ANY),
        out_shape=jax.ShapeDtypeStruct(out_rows + (L,), f32),
        scratch_shapes=[
            vmem((D, L), bf16),
            [vmem((D,), bf16)] * 6,
            vmem((2 * D, D), bf16),
            vmem((D, D), bf16),
            vmem((D, D), bf16),
            vmem((state_tiles, D // 2, LANES), u32),
            vmem((D, F), bf16),
            vmem((D, F), bf16),
            vmem((D, F), bf16),
            [vmem((feature_tiles, SUBS * PITCH, LANES), u32)] * (L // T),
            vmem((2, feature_tiles, 2, T, LANES), f32),
            [vmem((state_tiles, SUBS * PITCH, LANES), u32)] * (L // T),
            vmem((L // LANES,) + out_rows + (LANES,), f32),
            vmem((2,) + out_rows + (LANES,), f32),
            vmem((SUBS, L), f32),
            pltpu.SemaphoreType.DMA((27,)),
            pltpu.SemaphoreType.DMA((1,)),
        ],
        compiler_params=pltpu.CompilerParams(vmem_limit_bytes=96 * 1024 * 1024, disable_semaphore_checks=True),
        name="gm_s5_mod",
    )(jnp.transpose(A_x.reshape(L, D)), A_Lambda_re, A_Lambda_im, A_B_re, A_B_im, A_C_re, A_C_im, A_log_dt,
      A_Dskip, B_w_r, B_w_gate, B_w_up, jnp.transpose(B_w_down), gate_w)
    return jnp.transpose(out.reshape(D, L)).reshape(1, L, D)
```
